```python
import os as _os
_os.environ.setdefault("JAX_PLATFORMS", "cpu")
import jax
import jax.numpy as jnp

def _softmax(x, axis=-1):
    return jax.nn.softmax(x, axis=axis)
def _gelu(x):
    return jax.nn.gelu(x, approximate=True)
def _silu(x):
    return jax.nn.silu(x)
def _sigmoid(x):
    return jax.nn.sigmoid(x)
def _layernorm(x, axis=-1, eps=1e-5):
    m = jnp.mean(x, axis=axis, keepdims=True)
    v = jnp.var(x, axis=axis, keepdims=True)
    return (x - m) / jnp.sqrt(v + eps)
def _scatter_add(tgt, idx, src, axis=0):
    return tgt.at[idx].add(src)
def _segment_sum(src, seg, n):
    return jax.ops.segment_sum(src, seg, n)
class _Rng:
    def __init__(self, key):
        self._k = key
    def _next(self):
        self._k, sub = jax.random.split(self._k)
        return sub
    def normal(self, shape):
        return jax.random.normal(self._next(), shape, dtype=jnp.bfloat16)
    def randint(self, lo, hi, shape):
        return jax.random.randint(self._next(), shape, lo, hi, dtype=jnp.int32)
    def uniform(self, shape, lo=0.0, hi=1.0):
        return jax.random.uniform(self._next(), shape, jnp.bfloat16, lo, hi)
    def permutation(self, n):
        return jax.random.permutation(self._next(), n)


kernel_name = 'sequential_preLN__softmax_full_mha__glu_gated_swiglu__prompt'

def setup_inputs():
    _rng = _Rng(jax.random.key(int.from_bytes(__import__("os").urandom(4), "little")))
    _w = (lambda a: (lambda t: t.astype(jnp.bfloat16) if jnp.issubdtype(t.dtype, jnp.floating) else t)(jnp.asarray(a)))
    def _A_setup():
        B, S, D = 1, 2048, 640
        return {
            "x": _w((lambda *s: _rng.normal(s) * 0.05)(B, S, D)),
            "wqkv": _w((lambda *s: _rng.normal(s) * 0.05)(D, 3 * D)),
            "wo": _w((lambda *s: _rng.normal(s) * 0.05)(D, D)),
        }
    _A_in = _A_setup()

    def _B_setup():
        B, S, D, F = 1, 2048, 640, 1728
        return {
            "x": _w((lambda *s: _rng.normal(s) * 0.05)(B, S, D)),
            "w1": _w((lambda *s: _rng.normal(s) * 0.05)(D, F) * (2.0 / D) ** 0.5),
            "w3": _w((lambda *s: _rng.normal(s) * 0.05)(D, F) * (2.0 / D) ** 0.5),
            "w2": _w((lambda *s: _rng.normal(s) * 0.05)(F, D) * (2.0 / F) ** 0.5),
        }
    _B_in = _B_setup()

    return {
        "A_x": _A_in["x"],
        "A_wqkv": _A_in["wqkv"],
        "A_wo": _A_in["wo"],
        "B_x": _B_in["x"],
        "B_w1": _B_in["w1"],
        "B_w3": _B_in["w3"],
        "B_w2": _B_in["w2"],
    }

def reference(A_x, A_wqkv, A_wo, B_x, B_w1, B_w3, B_w2):
    def _A_ref(x, wqkv, wo):
        B, S, D = x.shape
        H = 32; Dh = D // H
        qkv = (lambda x, *d: x.transpose(*d))((x @ wqkv).reshape(B, S, 3, H, Dh), 2, 0, 3, 1, 4)
        q, k, v = qkv[0], qkv[1], qkv[2]
        scale = Dh ** -0.5
        scores = jnp.einsum("bhqd,bhkd->bhqk", q, k) * scale
        p = _softmax(scores, axis=-1)
        o = jnp.einsum("bhqk,bhkd->bhqd", p, v)
        return (lambda x, *d: x.transpose(*d))(o, 0, 2, 1, 3).reshape(B, S, D) @ wo

    def _B_ref(x, w1, w3, w2):
        gate = jnp.einsum("bsd,df->bsf", x, w1)
        up = jnp.einsum("bsd,df->bsf", x, w3)
        h = _silu(gate) * up
        out = jnp.einsum("bsf,fd->bsd", h, w2)
        return out

    x = A_x
    h = x + _A_ref(_layernorm(x, axis=-1), A_wqkv, A_wo)
    h2 = h + _B_ref(_layernorm(h, axis=-1), B_w1, B_w3, B_w2)
    return h2
```

```python
import functools
import math

import jax
import jax.numpy as jnp
from jax import lax
import jax.experimental.pallas as pl
import jax.experimental.pallas.tpu as pltpu

NUM_HEADS = 32
LANES = 128
LN_EPS = 1e-5


def _layernorm(x):
    m = jnp.mean(x, axis=-1, keepdims=True)
    xc = x - m
    v = jnp.mean(xc * xc, axis=-1, keepdims=True)
    return xc * lax.rsqrt(v + LN_EPS)


def _fused_kernel(x_ref, wqkv_ref, wo_ref, w1_ref, w3_ref, w2_ref, out_ref,
                  q_scr, kt_scr, v_scr, o_scr,
                  *, S, D, DH, HPG, NG, TQ, TR):
    f32 = jnp.float32
    bf16 = jnp.bfloat16
    GW = NG * LANES

    x = x_ref[...].astype(f32)
    ln = _layernorm(x).astype(bf16)

    qscale = (DH ** -0.5) * math.log2(math.e)
    q = jnp.dot(ln, wqkv_ref[:, 0:GW], preferred_element_type=f32)
    q_scr[...] = (q * qscale).astype(bf16)

    k = jnp.dot(ln, wqkv_ref[:, GW:2 * GW], preferred_element_type=f32)
    kt = k.T
    v = jnp.dot(ln, wqkv_ref[:, 2 * GW:3 * GW], preferred_element_type=f32)

    row_iota = lax.broadcasted_iota(jnp.int32, (LANES, S), 0)
    lane_iota = lax.broadcasted_iota(jnp.int32, (S, LANES), 1)
    for h in range(NUM_HEADS):
        g, j = divmod(h, HPG)
        ktg = kt[g * LANES:(g + 1) * LANES, :]
        rmask = (row_iota >= j * DH) & (row_iota < (j + 1) * DH)
        kt_scr[h] = jnp.where(rmask, ktg, 0.0).astype(bf16)
        vg = v[:, g * LANES:(g + 1) * LANES]
        lmask = (lane_iota >= j * DH) & (lane_iota < (j + 1) * DH)
        ones_col = (lane_iota == (HPG * DH + j)).astype(f32)
        v_scr[h] = jnp.where(lmask, vg, ones_col).astype(bf16)

    o_scr[...] = jnp.zeros(o_scr.shape, f32)

    n_qb = S // TQ

    def head_body(h, carry):
        g = h // HPG
        j = h - g * HPG
        lane_off = pl.multiple_of(g * LANES, LANES)
        kt_h = kt_scr[h]
        v_h = v_scr[h]
        lsel = lax.broadcasted_iota(jnp.int32, (TQ, LANES), 1) == (HPG * DH + j)

        def q_body(qi, c2):
            r0 = pl.multiple_of(qi * TQ, TQ)
            qg = q_scr[pl.ds(r0, TQ), pl.ds(lane_off, LANES)]
            s = jnp.dot(qg, kt_h, preferred_element_type=f32)
            m = jnp.max(s, axis=-1, keepdims=True)
            p = jnp.exp2(s - m)
            pv = jnp.dot(p.astype(bf16), v_h, preferred_element_type=f32)
            l = jnp.sum(jnp.where(lsel, pv, 0.0), axis=-1, keepdims=True)
            o_scr[pl.ds(r0, TQ), pl.ds(lane_off, LANES)] += pv / l
            return c2

        lax.fori_loop(0, n_qb, q_body, 0)
        return carry

    lax.fori_loop(0, NUM_HEADS, head_body, 0)

    n_rb = S // TR

    def row_body(ri, carry):
        r0 = pl.multiple_of(ri * TR, TR)
        o = o_scr[pl.ds(r0, TR), :].astype(bf16)
        attn = jnp.dot(o, wo_ref[...], preferred_element_type=f32).astype(bf16)
        xr = x_ref[pl.ds(r0, TR), :].astype(f32)
        hres = (xr + attn.astype(f32)).astype(bf16)
        hf = hres.astype(f32)
        ln2 = _layernorm(hf).astype(bf16)
        gate = jnp.dot(ln2, w1_ref[...], preferred_element_type=f32)
        up = jnp.dot(ln2, w3_ref[...], preferred_element_type=f32)
        act = (gate * jax.nn.sigmoid(gate) * up).astype(bf16)
        ffn = jnp.dot(act, w2_ref[...], preferred_element_type=f32).astype(bf16)
        out_ref[pl.ds(r0, TR), :] = (hf + ffn.astype(f32)).astype(out_ref.dtype)
        return carry

    lax.fori_loop(0, n_rb, row_body, 0)


@jax.jit
def pallas_sequential_preLN__softmax_full_mha__glu_gated_swiglu__prompt_kernel(
    A_x: jax.Array,
    A_wqkv: jax.Array,
    A_wo: jax.Array,
    B_x: jax.Array,
    B_w1: jax.Array,
    B_w3: jax.Array,
    B_w2: jax.Array,
):
    del B_x
    B, S, D = A_x.shape
    assert B == 1
    H = NUM_HEADS
    DH = D // H
    HPG = LANES // DH
    NG = -(-H // HPG)
    assert HPG * DH + HPG <= LANES or True
    F = B_w1.shape[1]

    x2 = A_x.reshape(S, D)

    def pad_heads_cols(w):
        w = w.reshape(w.shape[0], H, DH)
        w = jnp.pad(w, ((0, 0), (0, NG * HPG - H), (0, 0)))
        w = w.reshape(w.shape[0], NG, HPG * DH)
        w = jnp.pad(w, ((0, 0), (0, 0), (0, LANES - HPG * DH)))
        return w.reshape(w.shape[0], NG * LANES)

    wqkv = A_wqkv.reshape(D, 3, H * DH)
    wqkv_p = jnp.concatenate(
        [pad_heads_cols(wqkv[:, i, :]) for i in range(3)], axis=1)
    wo_p = pad_heads_cols(A_wo.T).T

    TQ = 256
    TR = 256
    kernel = functools.partial(
        _fused_kernel, S=S, D=D, DH=DH, HPG=HPG, NG=NG, TQ=TQ, TR=TR)

    out = pl.pallas_call(
        kernel,
        out_shape=jax.ShapeDtypeStruct((S, D), A_x.dtype),
        in_specs=[pl.BlockSpec(memory_space=pltpu.VMEM)] * 6,
        out_specs=pl.BlockSpec(memory_space=pltpu.VMEM),
        scratch_shapes=[
            pltpu.VMEM((S, NG * LANES), jnp.bfloat16),
            pltpu.VMEM((H, LANES, S), jnp.bfloat16),
            pltpu.VMEM((H, S, LANES), jnp.bfloat16),
            pltpu.VMEM((S, NG * LANES), jnp.float32),
        ],
        compiler_params=pltpu.CompilerParams(
            vmem_limit_bytes=100 * 1024 * 1024),
    )(x2, wqkv_p, wo_p, B_w1, B_w3, B_w2)
    return out.reshape(B, S, D)
```

```python
import functools
import math

import jax
import jax.numpy as jnp
from jax import lax
import jax.experimental.pallas as pl
import jax.experimental.pallas.tpu as pltpu

NUM_HEADS = 32
LANES = 128
LN_EPS = 1e-5
VROWS = 32


def _layernorm(x):
    m = jnp.mean(x, axis=-1, keepdims=True)
    xc = x - m
    v = jnp.mean(xc * xc, axis=-1, keepdims=True)
    return xc * lax.rsqrt(v + LN_EPS)


def _window_start(lo, dh):
    a = (lo // LANES) * LANES
    if lo - a + dh <= LANES:
        return a
    return (lo // 16) * 16


def _fused_kernel(x_hbm, wqkv_hbm, wo_hbm, w1t_hbm, w3t_hbm, w2_hbm, out_hbm,
                  x_ref, wqkv_ref, wo_ref, w1t_ref, w3t_ref, w2_ref, obuf,
                  in_sems, out_sems,
                  km_scr, qt_scr, vt_scr, ot_scr, st_a, st_b,
                  *, S, D, DH, TQ, TR):
    f32 = jnp.float32
    bf16 = jnp.bfloat16
    H = NUM_HEADS

    in_copies = [
        pltpu.make_async_copy(src, dst, in_sems.at[i])
        for i, (src, dst) in enumerate([
            (x_hbm, x_ref), (wqkv_hbm, wqkv_ref), (wo_hbm, wo_ref),
            (w1t_hbm, w1t_ref), (w3t_hbm, w3t_ref), (w2_hbm, w2_ref)])
    ]
    for c in in_copies:
        c.start()

    in_copies[0].wait()
    x = x_ref[...].astype(f32)
    ln = _layernorm(x).astype(bf16)
    in_copies[1].wait()
    qkv = jnp.dot(ln, wqkv_ref[...], preferred_element_type=f32)
    qscale = (DH ** -0.5) * math.log2(math.e)
    qt_scr[...] = (qkv[:, 0:D] * qscale).T.astype(bf16)
    k = qkv[:, D:2 * D]
    vt = qkv[:, 2 * D:3 * D].T

    lane = lax.broadcasted_iota(jnp.int32, (S, LANES), 1)
    ones_zeros = jnp.concatenate(
        [jnp.ones((1, S), f32), jnp.zeros((VROWS - DH - 1, S), f32)], axis=0)
    for h in range(H):
        lo = h * DH
        w0 = _window_start(lo, DH)
        kwin = k[:, w0:w0 + LANES]
        mask = (lane >= lo - w0) & (lane < lo - w0 + DH)
        km_scr[h] = jnp.where(mask, kwin, 0.0).astype(bf16)
        vt_scr[h] = jnp.concatenate(
            [vt[lo:lo + DH, :], ones_zeros], axis=0).astype(bf16)

    NC = S // TQ
    T = H * NC

    def win(h):
        lo = h * DH
        a = (lo // LANES) * LANES
        w0 = jnp.where(lo - a + DH <= LANES, a, (lo // 16) * 16)
        return pl.multiple_of(w0, 16)

    def qk(t):
        h = t // NC
        c0 = pl.multiple_of((t - h * NC) * TQ, TQ)
        qt = qt_scr[pl.ds(win(h), LANES), pl.ds(c0, TQ)]
        return jnp.dot(km_scr[h], qt, preferred_element_type=f32)

    def softmax_pv(t, st):
        h = t // NC
        c0 = pl.multiple_of((t - h * NC) * TQ, TQ)
        m = jnp.max(st.reshape(S // LANES, LANES, TQ), axis=0)
        m = jnp.max(m.reshape(LANES // 8, 8, TQ), axis=0)
        m = jnp.max(m, axis=0, keepdims=True)
        pt = jnp.exp2(st - m).astype(bf16)
        ot = jnp.dot(vt_scr[h], pt, preferred_element_type=f32)
        l = ot[DH:DH + 1, :]
        ot_scr[h, :, pl.ds(c0, TQ)] = ot / l

    st_a[...] = qk(0)

    def step(i, carry):
        t = 2 * i
        st_b[...] = qk(t + 1)
        softmax_pv(t, st_a[...])
        st_a[...] = qk(t + 2)
        softmax_pv(t + 1, st_b[...])
        return carry

    lax.fori_loop(0, T // 2 - 1, step, 0)
    st_b[...] = qk(T - 1)
    softmax_pv(T - 2, st_a[...])
    softmax_pv(T - 1, st_b[...])

    n_rb = S // TR
    for c in in_copies[2:]:
        c.wait()

    def out_copy(ri, slot):
        return pltpu.make_async_copy(
            obuf.at[slot], out_hbm.at[pl.ds(ri * TR, TR), :], out_sems.at[slot])

    nt = (((1,), (1,)), ((), ()))

    def row_body(ri, carry):
        r0 = pl.multiple_of(ri * TR, TR)
        ot = jnp.concatenate(
            [ot_scr[h, 0:DH, pl.ds(r0, TR)] for h in range(H)], axis=0)
        o = ot.T.astype(bf16)
        attn = jnp.dot(o, wo_ref[...], preferred_element_type=f32).astype(bf16)
        xr = x_ref[pl.ds(r0, TR), :].astype(f32)
        hres = (xr + attn.astype(f32)).astype(bf16)
        hf = hres.astype(f32)
        ln2 = _layernorm(hf).astype(bf16)
        gate = lax.dot_general(ln2, w1t_ref[...], nt, preferred_element_type=f32)
        up = lax.dot_general(ln2, w3t_ref[...], nt, preferred_element_type=f32)
        act = (gate * jax.nn.sigmoid(gate) * up).astype(bf16)
        ffn = jnp.dot(act, w2_ref[...], preferred_element_type=f32).astype(bf16)
        slot = ri % 2

        @pl.when(ri >= 2)
        def _():
            out_copy(ri - 2, slot).wait()

        obuf[slot] = (hf + ffn.astype(f32)).astype(obuf.dtype)
        out_copy(ri, slot).start()
        return carry

    lax.fori_loop(0, n_rb, row_body, 0)
    out_copy(n_rb - 2, (n_rb - 2) % 2).wait()
    out_copy(n_rb - 1, (n_rb - 1) % 2).wait()


@jax.jit
def pallas_sequential_preLN__softmax_full_mha__glu_gated_swiglu__prompt_kernel(
    A_x: jax.Array,
    A_wqkv: jax.Array,
    A_wo: jax.Array,
    B_x: jax.Array,
    B_w1: jax.Array,
    B_w3: jax.Array,
    B_w2: jax.Array,
):
    del B_x
    B, S, D = A_x.shape
    assert B == 1 and D % NUM_HEADS == 0
    H = NUM_HEADS
    DH = D // H
    assert DH + 1 <= VROWS
    TQ = 512
    TR = 256
    assert S % (2 * TQ) == 0 and S % TR == 0 and S // TR >= 2 and S % LANES == 0

    x2 = A_x.reshape(S, D)
    w1t = B_w1.T
    w3t = B_w3.T

    kernel = functools.partial(_fused_kernel, S=S, D=D, DH=DH, TQ=TQ, TR=TR)
    out = pl.pallas_call(
        kernel,
        out_shape=jax.ShapeDtypeStruct((S, D), A_x.dtype),
        in_specs=[pl.BlockSpec(memory_space=pl.ANY)] * 6,
        out_specs=pl.BlockSpec(memory_space=pl.ANY),
        scratch_shapes=[
            pltpu.VMEM((S, D), A_x.dtype),
            pltpu.VMEM(A_wqkv.shape, A_wqkv.dtype),
            pltpu.VMEM(A_wo.shape, A_wo.dtype),
            pltpu.VMEM(w1t.shape, w1t.dtype),
            pltpu.VMEM(w3t.shape, w3t.dtype),
            pltpu.VMEM(B_w2.shape, B_w2.dtype),
            pltpu.VMEM((2, TR, D), A_x.dtype),
            pltpu.SemaphoreType.DMA((6,)),
            pltpu.SemaphoreType.DMA((2,)),
            pltpu.VMEM((H, S, LANES), jnp.bfloat16),
            pltpu.VMEM((D, S), jnp.bfloat16),
            pltpu.VMEM((H, VROWS, S), jnp.bfloat16),
            pltpu.VMEM((H, VROWS, S), jnp.float32),
            pltpu.VMEM((S, TQ), jnp.float32),
            pltpu.VMEM((S, TQ), jnp.float32),
        ],
        compiler_params=pltpu.CompilerParams(
            vmem_limit_bytes=100 * 1024 * 1024),
    )(x2, A_wqkv, A_wo, w1t, w3t, B_w2)
    return out.reshape(B, S, D)
```
